```python
import os as _os
_os.environ.setdefault("JAX_PLATFORMS", "cpu")
import jax
import jax.numpy as jnp

def _softmax(x, axis=-1):
    return jax.nn.softmax(x, axis=axis)
def _gelu(x):
    return jax.nn.gelu(x, approximate=True)
def _silu(x):
    return jax.nn.silu(x)
def _sigmoid(x):
    return jax.nn.sigmoid(x)
def _layernorm(x, axis=-1, eps=1e-5):
    m = jnp.mean(x, axis=axis, keepdims=True)
    v = jnp.var(x, axis=axis, keepdims=True)
    return (x - m) / jnp.sqrt(v + eps)
def _scatter_add(tgt, idx, src, axis=0):
    return tgt.at[idx].add(src)
def _segment_sum(src, seg, n):
    return jax.ops.segment_sum(src, seg, n)
class _Rng:
    def __init__(self, key):
        self._k = key
    def _next(self):
        self._k, sub = jax.random.split(self._k)
        return sub
    def normal(self, shape):
        return jax.random.normal(self._next(), shape, dtype=jnp.bfloat16)
    def randint(self, lo, hi, shape):
        return jax.random.randint(self._next(), shape, lo, hi, dtype=jnp.int32)
    def uniform(self, shape, lo=0.0, hi=1.0):
        return jax.random.uniform(self._next(), shape, jnp.bfloat16, lo, hi)
    def permutation(self, n):
        return jax.random.permutation(self._next(), n)


kernel_name = 'sequential_preLN__mha_block__dense_activation_squared_relu__prompt'

def setup_inputs():
    _rng = _Rng(jax.random.key(int.from_bytes(__import__("os").urandom(4), "little")))
    _w = (lambda a: (lambda t: t.astype(jnp.bfloat16) if jnp.issubdtype(t.dtype, jnp.floating) else t)(jnp.asarray(a)))
    def _A_setup():
        B, S, D, H = 1, 2048, 448, 16
        return {
            "x": _w((lambda *s: _rng.normal(s) * 0.05)(B, S, D)),
            "wqkv": _w((lambda *s: _rng.normal(s) * 0.05)(D, 3 * D)),
            "wo": _w((lambda *s: _rng.normal(s) * 0.05)(D, D)),
        }
    _A_in = _A_setup()

    def _B_setup():
        B, S, D, F = 1, 2048, 448, 1792
        return {
            "x": _w((lambda *s: _rng.normal(s) * 0.05)(B, S, D)),
            "w1": _w((lambda *s: _rng.normal(s) * 0.05)(D, F)),
            "b1": _w((lambda *s: _rng.normal(s) * 0.05)(F)),
            "w2": _w((lambda *s: _rng.normal(s) * 0.05)(F, D)),
            "b2": _w((lambda *s: _rng.normal(s) * 0.05)(D)),
        }
    _B_in = _B_setup()

    return {
        "A_x": _A_in["x"],
        "A_wqkv": _A_in["wqkv"],
        "A_wo": _A_in["wo"],
        "B_x": _B_in["x"],
        "B_w1": _B_in["w1"],
        "B_b1": _B_in["b1"],
        "B_w2": _B_in["w2"],
        "B_b2": _B_in["b2"],
    }

def reference(A_x, A_wqkv, A_wo, B_x, B_w1, B_b1, B_w2, B_b2):
    def _A_ref(x, wqkv, wo):
        B, S, D = x.shape
        H = 16
        Dh = D // H
        qkv = (lambda x, *d: x.transpose(*d))((x @ wqkv).reshape(B, S, 3, H, Dh), 2, 0, 3, 1, 4)
        q, k, v = qkv[0], qkv[1], qkv[2]
        scores = jnp.einsum("bhqd,bhkd->bhqk", q, k) * (Dh ** -0.5)
        p = _softmax(scores, axis=-1)
        o = jnp.einsum("bhqk,bhkd->bhqd", p, v)
        return (lambda x, *d: x.transpose(*d))(o, 0, 2, 1, 3).reshape(B, S, D) @ wo

    def _B_ref(x, w1, b1, w2, b2):
        h = jnp.einsum("bsd,df->bsf", x, w1) + b1
        zero = jnp.zeros_like(h)
        r = jnp.where(h > zero, h, zero)
        h = r * r
        out = jnp.einsum("bsf,fd->bsd", h, w2) + b2
        return out

    x = A_x
    h = x + _A_ref(_layernorm(x, axis=-1), A_wqkv, A_wo)
    h2 = h + _B_ref(_layernorm(h, axis=-1), B_w1, B_b1, B_w2, B_b2)
    return h2
```

```python
import functools
import math
import jax
import jax.numpy as jnp
from jax import lax
import jax.experimental.pallas as pl
import jax.experimental.pallas.tpu as pltpu

S, D, H, DH, F = 2048, 448, 16, 28, 1792
HP = 32
TQ = 512
NQ = S // TQ
R0 = 512
KC = 256
HPI = 4
EPS = 1e-5
QSCALE = (DH ** -0.5) * math.log2(math.e)
f32, bf16 = jnp.float32, jnp.bfloat16
DP = 512
NW = 2 * D + H * HP


def _lnT(x):
    mu = jnp.mean(x, axis=0, keepdims=True)
    xc = x - mu
    var = jnp.mean(xc * xc, axis=0, keepdims=True)
    return xc * lax.rsqrt(var + EPS)


def kernel(xT_ref, wqkv_ref, wo_ref, w1_ref, b1_ref, w2T_ref, b2_ref, o_ref,
           tmp_s, wT_s, woT_s, w1T_s, b2c_s, qT_s, k_s, vT_s, sA, sB, mA, mB, oT_s):
    i = pl.program_id(0)

    def qmask(blk, t, j):
        qt = qT_s[t, :, pl.ds(pl.multiple_of(blk * TQ, TQ), TQ)]
        row = lax.broadcasted_iota(jnp.int32, (128, TQ), 0)
        lo = j * DH
        return jnp.where((row >= lo) & (row < lo + DH), qt, jnp.zeros_like(qt))

    def step(qm, t_next, s_next, m_next, h, s_cur, m_cur):
        mx = None
        acc = None
        if h is not None:
            m = m_cur[...]
        for c in range(S // KC):
            rows = slice(c * KC, (c + 1) * KC)
            if qm is not None:
                s = jnp.dot(k_s[t_next, rows, :], qm, preferred_element_type=f32)
                s_next[rows, :] = s
                cm = jnp.max(s.reshape(KC // 8, 8, TQ), axis=0)
                mx = cm if mx is None else jnp.maximum(mx, cm)
            if h is not None:
                p = jnp.exp2(s_cur[rows, :] - m).astype(bf16)
                o = jnp.dot(vT_s[h, :, rows], p, preferred_element_type=f32)
                acc = o if acc is None else acc + o
        if qm is not None:
            m_next[...] = jnp.max(mx, axis=0, keepdims=True)
        if h is not None:
            l = acc[DH:DH + 1, :]
            oT_s[h] = (acc * (1.0 / l)).astype(bf16)

    @pl.when(i == 0)
    def _():
        w = wqkv_ref[...].astype(f32)
        w = jnp.concatenate([w, jnp.zeros((DP - D, 3 * D), f32)], axis=0)
        w = jnp.concatenate([w, jnp.zeros((DP, 64), f32)], axis=1)
        tmp_s[0:1408, :] = w.T
        wT_s[0:2 * D, :] = tmp_s[0:2 * D, :].astype(bf16)
        for h in range(H):
            blk = jnp.concatenate([tmp_s[2 * D + DH * h:2 * D + DH * (h + 1), :],
                                   jnp.zeros((HP - DH, DP), f32)], axis=0)
            wT_s[2 * D + HP * h:2 * D + HP * (h + 1), :] = blk.astype(bf16)
        wo = wo_ref[...].astype(f32)
        wo = jnp.concatenate([wo, jnp.zeros((D, DP - D), f32)], axis=1)
        tmp_s[0:D, :] = wo
        for h in range(H):
            blk = jnp.concatenate([tmp_s[DH * h:DH * (h + 1), :],
                                   jnp.zeros((HP - DH, DP), f32)], axis=0)
            tmp_s[512 + HP * h:512 + HP * (h + 1), :] = blk
        woT_s[...] = tmp_s[512:1024, :].T[0:D, :].astype(bf16)
        rr = lax.broadcasted_iota(jnp.int32, (DP - D, F), 0)
        brow = jnp.where(rr == 0, jnp.broadcast_to(b1_ref[...].astype(f32), (DP - D, F)), 0.0)
        w1a = jnp.concatenate([w1_ref[...].astype(f32), brow], axis=0)
        w1T_s[...] = w1a.T.astype(bf16)
        b2r = jnp.concatenate([b2_ref[...].astype(f32), jnp.zeros((1, DP - D), f32)], axis=1)
        b2c_s[...] = jnp.broadcast_to(b2r, (128, DP)).T[0:D, :]
        qT_s[:, 112:128, :] = jnp.zeros((4, 16, S), bf16)

        def chunk(c, carry):
            cols = pl.ds(pl.multiple_of(c * R0, R0), R0)
            xn = _lnT(xT_ref[:, cols].astype(f32)).astype(bf16)
            r = jnp.dot(wT_s[:, 0:D], xn, preferred_element_type=f32)
            for t in range(4):
                qT_s[t, 0:112, cols] = (r[112 * t:112 * (t + 1), :] * QSCALE).astype(bf16)
                kt = r[D + 112 * t:D + 112 * t + 128, :]
                k_s[t, cols, :] = kt.T.astype(bf16)
            vT = r[2 * D:, :]
            rr = lax.broadcasted_iota(jnp.int32, (H * HP, R0), 0)
            vT = jnp.where(rr % HP == DH, 1.0, vT).astype(bf16)
            vT_s[:, :, cols] = vT.reshape(H, HP, R0)
            return carry
        lax.fori_loop(0, S // R0, chunk, 0)
        step(qmask(0, 0, 0), 0, sA, mA, None, None, None)

    bufs = [(sA, mA), (sB, mB)]

    def group(t, carry):
        for j in range(HPI):
            h = t * 4 + j
            cur = bufs[j % 2]
            nxt = bufs[(j + 1) % 2]
            if j < 3:
                qm = qmask(i, t, j + 1)
                tn = t
            else:
                last = t == 3
                nb = jnp.where(last, jnp.minimum(i + 1, NQ - 1), i)
                tn = jnp.where(last, 0, t + 1)
                qm = qmask(nb, tn, 0)
            step(qm, tn, nxt[0], nxt[1], h, cur[0], cur[1])
        return carry
    lax.fori_loop(0, 4, group, 0)

    cols = pl.ds(pl.multiple_of(i * TQ, TQ), TQ)
    oT = oT_s[...].reshape(H * HP, TQ)
    hT = xT_ref[:, cols].astype(f32) + jnp.dot(woT_s[...], oT, preferred_element_type=f32)
    hn = _lnT(hT)
    rr = lax.broadcasted_iota(jnp.int32, (16, TQ), 0)
    hna = jnp.concatenate([hn, jnp.where(rr == 0, 1.0, 0.0)], axis=0).astype(bf16)
    a = jnp.dot(w1T_s[:, 0:D + 16], hna, preferred_element_type=f32)
    a = jnp.maximum(a, 0.0)
    a = (a * a).astype(bf16)
    y = jnp.dot(w2T_ref[...], a, preferred_element_type=f32)
    b2 = b2c_s[...]
    b2 = jnp.concatenate([b2] * (TQ // 128), axis=1)
    o_ref[...] = (hT + y + b2).astype(o_ref.dtype)


@jax.jit
def pallas_sequential_preLN__mha_block__dense_activation_squared_relu__prompt_kernel(A_x, A_wqkv, A_wo, B_x, B_w1, B_b1, B_w2, B_b2):
    full = lambda shape: pl.BlockSpec(shape, lambda i: (0,) * len(shape))
    outT = pl.pallas_call(
        kernel,
        grid=(NQ,),
        in_specs=[
            pl.BlockSpec((None, D, S), lambda i: (0, 0, 0)),
            full((D, 3 * D)), full((D, D)), full((D, F)), full((1, F)), full((D, F)), full((1, D)),
        ],
        out_specs=pl.BlockSpec((None, D, TQ), lambda i: (0, 0, i)),
        out_shape=jax.ShapeDtypeStruct((1, D, S), bf16),
        scratch_shapes=[
            pltpu.VMEM((1408, DP), f32),
            pltpu.VMEM((NW, DP), bf16),
            pltpu.VMEM((D, DP), bf16),
            pltpu.VMEM((F, DP), bf16),
            pltpu.VMEM((D, 128), f32),
            pltpu.VMEM((4, 128, S), bf16),
            pltpu.VMEM((4, S, 128), bf16),
            pltpu.VMEM((H, HP, S), bf16),
            pltpu.VMEM((S, TQ), f32),
            pltpu.VMEM((S, TQ), f32),
            pltpu.VMEM((1, TQ), f32),
            pltpu.VMEM((1, TQ), f32),
            pltpu.VMEM((H, HP, TQ), bf16),
        ],
        compiler_params=pltpu.CompilerParams(
            dimension_semantics=("arbitrary",),
            vmem_limit_bytes=100 * 1024 * 1024),
    )(jnp.swapaxes(A_x, 1, 2), A_wqkv, A_wo, B_w1, B_b1.reshape(1, F), B_w2.T, B_b2.reshape(1, D))
    return jnp.swapaxes(outT, 1, 2)
```

```python
import math

import jax
import jax.numpy as jnp
from jax import lax
import jax.experimental.pallas as pl
import jax.experimental.pallas.tpu as pltpu

S, D, H, DH, F = 2048, 448, 16, 28, 1792
HP = 32
TQ = 256
NQ = S // TQ
NT = TQ // 128
HPI = 16
R0 = 512
KC = 256
NC = S // KC
EPS = 1e-5
QSCALE = (DH ** -0.5) * math.log2(math.e)
f32, bf16, u32 = jnp.float32, jnp.bfloat16, jnp.uint32
DP = 512
NP = DH // 2
CROW = 4 * DH
BIG = 2.0 ** 100
TINY = 2.0 ** -40

NV = 240
RV = 2
NVP = NV // (8 * RV)
NVT = -(-NV // 128) * 128
NMS = H * NVP * NP
H0 = 5
PRE = 3
LAG = 3
TAIL = 'a00_p_p_a01_p_a10_a11_b_q_q_q'
NGR = (S - NV) // 16
GB = [n * NGR // NC for n in range(NC + 1)]
_ODD = [sum((GB[m + 1] - GB[m]) % 2 for m in range(n)) % 2 for n in range(NC)]
MCH = [(NV + 16 * GB[n], NV + 16 * GB[n + 1]) for n in range(NC)]

LAT = 130
LAT0 = 100
RATIO = 1.1
R2 = 0.8
RO = 0.7
OOFF = 100
TSTART = 100
TEND = 400
PAUSE0 = 300
PAUSE1 = 1000
P0S = 400
P0E = 250
R5R = 0.01
T_ATT = H * (8 * NGR + 32 * NC)
T_FFN = 7616

A_P = (0, S // 2)
A_PV = S
A_C = A_PV + H * NV // 2
A_QB = A_C + H * 8
A_HY = A_QB + 2 * DH * 8
A_HD = A_HY + D
A_ACT = A_HD + D
A_ACC = A_ACT + F // 2
A_QC = A_ACC + HP
A_QN = A_QC + 224
A_END = A_QN + 224


def _spread(n, segs):
    tot = sum((b - a) * r for a, b, r in segs)
    out = []
    for ms in range(n):
        w = tot * ms / n
        for a, b, r in segs:
            if w < (b - a) * r:
                out.append(a + w / r)
                break
            w -= (b - a) * r
    return out


def _ms_times():
    f2 = T_ATT + 896 + 2 * F
    to = T_ATT - PRE * NGR - 32 * LAG + OOFF
    return _spread(NMS, [(TSTART, to, 1.0), (to, T_ATT + PAUSE0, RO), (T_ATT + PAUSE1, f2 + 100, RATIO),
                         (f2 + 100, f2 + 4 * D + 100, RATIO * R2),
                         (f2 + 4 * D + 100, T_ATT + T_FFN - TEND, RATIO)])


def _p0_times(n0):
    t0 = 448 + 3 * F
    tb = t0 + 5 * F
    return _spread(n0, [(t0 + P0S, tb - P0E, 1.0), (tb + 150, t0 + 6 * F, R5R)])


def pk(x):
    return pltpu.bitcast(x, u32)


def upk(x):
    return pltpu.bitcast(x, bf16)


def asf(x):
    return lax.bitcast_convert_type(x, f32)


def asu(x):
    return lax.bitcast_convert_type(x, u32)


def dot(a, b):
    return jnp.dot(a, b, preferred_element_type=f32)


def pack_pairs(ke, ko):
    lo = asu(ke.astype(bf16).astype(f32)) >> 16
    bits = asu(ko)
    sign = bits & jnp.uint32(0x80000000)
    mag = (bits & jnp.uint32(0x7fffffff)).astype(jnp.int32)
    hi = jnp.maximum(mag - lo.astype(jnp.int32) + 0x8000, 0).astype(u32) & jnp.uint32(0x7fff0000)
    return sign | hi | lo


def _padT(w):
    r, c = w.shape
    rp, cp = -(-r // 128) * 128, -(-c // 128) * 128
    if rp != r:
        w = jnp.concatenate([w, jnp.zeros((rp - r, c), w.dtype)], axis=0)
    if cp != c:
        w = jnp.concatenate([w, jnp.zeros((rp, cp - c), w.dtype)], axis=1)
    return w.T


def first_row(rows, cols, val=1.0):
    return jnp.where(lax.broadcasted_iota(jnp.int32, (rows, cols), 0) == 0, val, 0.0)


def fold8(v, op):
    return op(v.reshape(v.shape[0] // 8, 8, v.shape[1]), axis=0)


def kernel(xT_hbm, wqkv_hbm, wo_hbm, w1_hbm, b1_hbm, w2T_hbm, b2_hbm, o_ref,
           xT_ref, wqkv_ref, wo_ref, w1_ref, b1_ref, w2T_ref, b2_ref, sems,
           wT_s, woT_s, w1T_s, b2c_s, qT_s, k_s, vT_s, ar, oT_s, kp_s, z_s, kt_s, fs_s, mu_s):
    i = pl.program_id(0)

    def gate(v, tok, on):
        if tok is None:
            return v
        r, c = v.shape
        tok = lax.bitcast_convert_type(tok, v.dtype)
        return jnp.concatenate(
            [jnp.concatenate([jnp.where(on, v[a:a + 8, b:b + 128], tok) for b in range(0, c, 128)], axis=1)
             for a in range(0, r, 8)], axis=0)

    def fetch_q(blk):
        cols = pl.ds(pl.multiple_of(blk * TQ, TQ), TQ)
        for t in range(4):
            ar[A_QN + 56 * t:A_QN + 56 * (t + 1), :] = asf(qT_s[t, :, cols])

    def qmask(src, h):
        t, j = divmod(h, 4)
        lo = j * DH
        w0 = (lo // 16) * 16
        w1 = -(-(lo + DH) // 16) * 16
        qt = asu(ar[src + 56 * t + w0 // 2:src + 56 * t + w1 // 2, :])
        row = lax.broadcasted_iota(jnp.int32, qt.shape, 0) + w0 // 2
        qt = jnp.where((row >= lo // 2) & (row < (lo + DH) // 2), qt, jnp.zeros_like(qt))
        parts = [jnp.zeros((w0, TQ), bf16), upk(qt), jnp.zeros((CROW - w1, TQ), bf16),
                 upk(asu(ar[A_C + 8 * h:A_C + 8 * h + 8, :]))]
        return jnp.concatenate([x for x in parts if x.shape[0]], axis=0)

    def set_shift(h, s):
        c = jnp.max(fold8(s, jnp.max), axis=0, keepdims=True).astype(bf16).astype(f32)
        c = jnp.broadcast_to(c, (8, TQ))
        row = lax.broadcasted_iota(jnp.int32, (8, TQ), 0)
        ar[A_C + 8 * h:A_C + 8 * h + 8, :] = asf(jnp.where(row == 0, asu(-c) >> 16, jnp.uint32(0)))
        return c

    def qk_chunk(qm, h, c):
        r0, r1 = MCH[c]
        rm = r0 + 16 * (((r1 - r0) // 16 + (_ODD[c] + h * NGR) % 2) // 2)
        halves = [jnp.concatenate([dot(upk(k_s[4 * n + h // 4, a // 2:b // 2, :]), qm[:, n * 128:(n + 1) * 128])
                                   for n in range(NT)], axis=1) for a, b in ((r0, rm), (rm, r1))]
        p = jnp.exp2(jnp.concatenate(halves, axis=0)).astype(bf16)
        ar[A_P[h % 2] + r0 // 2:A_P[h % 2] + r1 // 2, :] = asf(pk(p))
        return halves[0]

    def make_stream(seq, after, prebuilt, times, free, lat):
        vs = dict(next=0, free=free, shift=set(), done=set())
        on = z_s[...] == 0
        toks = []
        clk = dict(now=0)

        def qb_rows(h, d):
            r0 = A_QB + ((h % 2) * DH + d) * 8
            return slice(r0, r0 + 8)

        def qb_build(h, src, p, tok):
            rw = 56 * (h // 4) + (h % 4) * NP + p
            qt = gate(asu(ar[src + rw // 8 * 8:src + rw // 8 * 8 + 8, :]), tok, on)
            qq = jnp.broadcast_to(qt[rw % 8:rw % 8 + 1, :], (8, TQ))
            ar[qb_rows(h, 2 * p), :] = asf(qq << 16)
            ar[qb_rows(h, 2 * p + 1), :] = asf(qq & jnp.uint32(0xffff0000))

        def tok_at(t):
            best = None
            for tt, v in toks:
                if tt <= t and (best is None or tt > best[0]):
                    best = (tt, v)
            return None if best is None else best[1]

        def micro(ms):
            pos, rem = divmod(ms, NVP * NP)
            h = seq[pos][0]
            pc, p = divmod(rem, NP)
            tok = tok_at(times[ms])
            kv = gate(kp_s[p, pc * RV * 8:(pc + 1) * RV * 8, :], tok, on)
            w = jnp.broadcast_to(kv[:, h:h + 1], (RV * 8, 128))
            for e, a in enumerate((asf(w << 16), asf(w))):
                b = ar[qb_rows(h, 2 * p + e), :]
                tt = jnp.concatenate([a] * NT, axis=1).reshape(RV, 8, TQ) * b[None]
                vs['acc'] = tt if p == 0 and e == 0 else vs['acc'] + tt
            nxt = seq[pos + 1] if pos + 1 < len(seq) else after
            if rem % NVP == 0:
                qb_build(*nxt, rem // NVP, tok)
            if p == NP - 1:
                assert h in vs['free'], (h, ms)
                if pc == 0:
                    vs['c'] = set_shift(h, vs['acc'].reshape(RV * 8, TQ))
                    vs['shift'].add(h)
                pv = jnp.exp2(vs['acc'] - vs['c'][None]).reshape(RV * 8, TQ).astype(bf16)
                r0 = A_PV + (h * NV + pc * RV * 8) // 2
                ar[r0:r0 + RV * 4, :] = asf(pk(pv))
                if pc == NVP - 1:
                    vs['done'].add(h)

        def issued(res, cost, ntile=1):
            if res is not None:
                for n in range(ntile):
                    for u in range(res.shape[0] // 16):
                        toks.append((clk['now'] + res.shape[0] * n + 16 * u + lat,
                                     res[16 * u:16 * u + 8, 128 * n:128 * (n + 1)]))
            clk['now'] += cost
            while vs['next'] < len(times) and times[vs['next']] < clk['now'] + lat:
                micro(vs['next'])
                vs['next'] += 1

        if not prebuilt:
            for p in range(NP):
                qb_build(*seq[0], p, None)
        return vs, issued

    @pl.when(i == 0)
    def _():
        srcs = [
            (wqkv_hbm.at[:, 0:256], wqkv_ref.at[:, 0:256]),
            (xT_hbm.at[0, :, 0:R0], xT_ref.at[:, 0:R0]),
            (wqkv_hbm.at[:, 256:512], wqkv_ref.at[:, 256:512]),
            (wqkv_hbm.at[:, 512:3 * D], wqkv_ref.at[:, 512:3 * D]),
            (xT_hbm.at[0, :, R0:S], xT_ref.at[:, R0:S]),
            (wo_hbm, wo_ref), (w1_hbm, w1_ref), (b1_hbm, b1_ref), (b2_hbm, b2_ref),
            (w2T_hbm, w2T_ref),
        ]
        cps = [pltpu.make_async_copy(a, b, sems.at[n]) for n, (a, b) in enumerate(srcs)]
        for cp in cps:
            cp.start()
        c_wa1, c_x0, c_wa2, c_wb, c_x1, c_wo, c_w1, c_b1, c_b2, c_w2 = cps
        hook, mus = [], []

        def ln_chunk(c):
            x = xT_ref[:, c * R0:(c + 1) * R0].astype(f32)
            mu = jnp.mean(x, axis=0, keepdims=True)
            mus.append(mu)
            xc = x - mu
            rs = lax.rsqrt(jnp.mean(xc * xc, axis=0, keepdims=True) + EPS)
            return xc.astype(bf16), rs

        def proj(r0, r1, xc):
            r = dot(upk(wT_s[r0 // 2:r1 // 2, 0:D]), xc)
            if hook:
                hook[0](r, (r1 - r0) * (R0 // 128), R0 // 128)
            return r

        def q_part(c, xn, ts):
            r0, r1 = 112 * ts[0], 112 * (ts[-1] + 1)
            r = proj(r0, r1, xn[0]) * (xn[1] * QSCALE)
            for t in ts:
                qT_s[t, :, c * R0:(c + 1) * R0] = pk(r[112 * t - r0:112 * (t + 1) - r0, :].astype(bf16))

        def k_part(c, xn):
            r = proj(D, 2 * D, xn[0]) * xn[1]
            if c == 0:
                for n in range(NVT // 128):
                    kt_s[n] = r[:, n * 128:(n + 1) * 128]
                for p in range(NP):
                    for n in range(NVT // 128):
                        w = pack_pairs(kt_s[n, pl.ds(2 * p, H, stride=DH), :],
                                       kt_s[n, pl.ds(2 * p + 1, H, stride=DH), :])
                        w = jnp.concatenate([w, jnp.zeros((128 - H, 128), u32)], axis=0)
                        kp_s[p, n * 128:(n + 1) * 128, :] = w.T
            for t in range(4):
                kt = jnp.concatenate([r[112 * t:112 * (t + 1), :], first_row(16, R0)], axis=0)
                kk = pk(kt.T.astype(bf16))
                for n in range(NT):
                    k_s[4 * n + t, c * R0 // 2:(c + 1) * R0 // 2, :] = kk

        def v_part(c, xn, hs):
            r0, r1 = DH * hs[0], DH * (hs[-1] + 1)
            r = proj(2 * D + r0, 2 * D + r1, xn[0]) * xn[1]
            for h in hs:
                blk = jnp.concatenate([r[DH * h - r0:DH * (h + 1) - r0, :], first_row(HP - DH, R0)], axis=0)
                vT_s[h, :, c * R0:(c + 1) * R0] = pk(blk.astype(bf16))

        def wt_part(c0, c1):
            wT = pk(_padT(wqkv_ref[:, c0:c1].astype(f32)).astype(bf16))
            wT_s[c0 // 2:c0 // 2 + wT.shape[0], :] = wT

        z_s[...] = jnp.zeros((8, 128), u32)
        c_wa1.wait()
        wt_part(0, 256)
        c_x0.wait()
        xn0 = ln_chunk(0)
        q_part(0, xn0, [0])
        c_wa2.wait()
        q_part(0, xn0, [1])
        wt_part(256, 512)
        q_part(0, xn0, [2])
        c_wb.wait()
        q_part(0, xn0, [3])
        wt_part(512, 3 * D)
        k_part(0, xn0)
        v_part(0, xn0, list(range(0, 12)))
        c_x1.wait()
        c_wo.wait()
        fetch_q(0)
        vs0, issued0 = make_stream([(h, A_QN) for h in range(H0)], (H0, A_QN), False,
                                   _p0_times(H0 * NVP * NP), set(range(H)), LAT0)
        hook.append(issued0)
        v_part(0, xn0, list(range(12, 16)))
        wo = wo_ref[...].astype(f32)
        parts = []
        for h in range(H):
            parts += [wo[DH * h:DH * (h + 1), :], jnp.zeros((HP - DH, D), f32)]
        woT_s[...] = pk(_padT(jnp.concatenate(parts, axis=0))[0:D, :].astype(bf16))
        xns = {}
        for c in range(1, S // R0):
            xns[c] = ln_chunk(c)
            k_part(c, xns[c])
        for c in range(1, S // R0):
            q_part(c, xns[c], [0, 1, 2, 3])
            if c == S // R0 - 1:
                c_w1.wait()
                c_b1.wait()
                c_b2.wait()
                c_w2.wait()
                mu_s[...] = jnp.concatenate(mus, axis=1)
                brow = first_row(DP - D, F, b1_ref[...].astype(f32).reshape(1, F))
                w1a = jnp.concatenate([w1_ref[...].astype(f32), brow], axis=0)
                w1T_s[...] = pk(w1a.T.astype(bf16))
            v_part(c, xns[c], list(range(H)))
        assert vs0['next'] == H0 * NVP * NP
        b2 = b2_ref[...].astype(f32).reshape(1, D)
        b2c_s[...] = _padT(jnp.broadcast_to(b2, (128, D)))[0:D, :]
        qm = qmask(A_QN, 0)
        for c in range(PRE):
            qk_chunk(qm, 0, c)

    st = dict(qm=qmask(A_QN, 0), bad=None)
    ar[A_QC:A_QC + 224, :] = ar[A_QN:A_QN + 224, :]
    fetch_q(jnp.minimum(i + 1, NQ - 1))
    vs, issued = make_stream([(h, A_QC) for h in range(H0, H)] + [(h, A_QN) for h in range(H0)],
                             (H0, A_QN), True, _ms_times(), set(range(H0, H)), LAT)

    def do_qk(n):
        hq, c = divmod(n, NC)
        if c == 0:
            assert hq < H0 or hq % H in vs['shift'], hq
            st['qm'] = qmask(A_QC if hq < H else A_QN, hq % H)
        first = qk_chunk(st['qm'], hq % H, c)
        issued(first, (MCH[c][1] - MCH[c][0]) // 2)

    def do_pv(n):
        h, pos = divmod(n, NC)
        order = [1, 2, 3, 4, 5, 6, 7, 0] if h < H - 1 else [1, 2, 3, 4, 5, 0, 6, 7]
        c = order[pos]
        base = A_P[h % 2]
        if c == 0:
            assert h < H0 or h in vs['done'], h
            p = ar[A_PV + h * NV // 2:A_PV + (h + 1) * NV // 2, :]
            if NV < KC:
                p = jnp.concatenate([p, ar[base + NV // 2:base + KC // 2, :]], axis=0)
            vs['free'].add(h)
        else:
            p = ar[base + c * KC // 2:base + (c + 1) * KC // 2, :]
        acc = dot(upk(vT_s[h, :, c * KC:(c + 1) * KC]), upk(asu(p)))
        if pos > 0:
            acc = ar[A_ACC:A_ACC + HP, :] + acc
        if pos < NC - 1:
            ar[A_ACC:A_ACC + HP, :] = acc
        else:
            l = acc[DH:DH + 1, :]
            oT_s[h] = pk((acc * (1.0 / l)).astype(bf16))
            bad = fold8(jnp.where(jnp.abs(acc) <= BIG, 0.0, 1.0), jnp.max)
            bad = jnp.maximum(bad, jnp.where(l >= TINY, 0.0, 1.0))
            st['bad'] = bad if st['bad'] is None else jnp.maximum(st['bad'], bad)
        issued(None, 32)

    shift, sums = {}, {}

    def do_op(k0, k1, n0, n1, r0, r1):
        lanes = slice(n0 * 128, n1 * 128)
        oT = upk(oT_s[k0 // HP:k1 // HP, :, lanes].reshape((k1 - k0) // 2, (n1 - n0) * 128))
        r = dot(upk(woT_s[r0 // 2:r1 // 2, k0:k1]), oT)
        issued(r, (r1 - r0) * ((k1 - k0) // 128) * (n1 - n0) // 4)
        if k0 == 0:
            xcols = pl.ds(pl.multiple_of(i * TQ + n0 * 128, 128), 128)
            shift[n0] = mu_s[0:1, xcols]
            ar[A_HD + r0:A_HD + r1, lanes] = (xT_ref[r0:r1, xcols].astype(f32) - shift[n0]) + r
        else:
            d = ar[A_HD + r0:A_HD + r1, lanes] + r
            ar[A_HD + r0:A_HD + r1, lanes] = d
            sums[r0] = (fold8(d, jnp.sum), fold8(d * d, jnp.sum))

    def ln2(n):
        lanes = slice(n * 128, (n + 1) * 128)
        s1 = sum(v[0][:, lanes] for v in sums.values())
        s2 = sum(v[1][:, lanes] for v in sums.values())
        mu = jnp.sum(s1, axis=0, keepdims=True) * (1.0 / D)
        var = jnp.maximum(jnp.sum(s2, axis=0, keepdims=True) * (1.0 / D) - mu * mu, 0.0)
        hn = (ar[A_HD:A_HD + D, lanes] - mu) * lax.rsqrt(var + EPS)
        return jnp.concatenate([hn, first_row(16, 128)], axis=0).astype(bf16)

    npv = 0
    for n in range(PRE, H * NC):
        do_qk(n)
        while npv <= n - LAG:
            do_pv(npv)
            npv += 1
    nqk = H * NC
    HD = D // 2
    for item in TAIL.split('_'):
        if item == 'q':
            do_qk(nqk)
            nqk += 1
        elif item == 'p':
            do_pv(npv)
            npv += 1
        elif item[0] == 'a':
            n, hf = int(item[1]), int(item[2])
            do_op(0, 384, n, n + 1, hf * HD, (hf + 1) * HD)
        elif item == 'b':
            assert npv == H * NC
            for hf in range(2):
                do_op(384, 512, 0, NT, hf * HD, (hf + 1) * HD)
    assert nqk == H * NC + PRE
    unsafe = jnp.max(st['bad']) > 0.0

    for n in range(NT):
        lanes = slice(n * 128, (n + 1) * 128)
        a = dot(upk(w1T_s[:, 0:D + 16]), ln2(n))
        issued(a, F)
        ar[A_HY:A_HY + D, lanes] = ar[A_HD:A_HD + D, lanes] + (b2c_s[...] + shift[n])
        a = jnp.maximum(a, 0.0)
        ar[A_ACT:A_ACT + F // 2, lanes] = asf(pk((a * a).astype(bf16)))

    def y_round(k0, k1, n0, n1, final):
        lanes = slice(n0 * 128, n1 * 128)
        r = dot(w2T_ref[:, k0:k1], upk(asu(ar[A_ACT + k0 // 2:A_ACT + k1 // 2, lanes])))
        issued(r, D)
        r = ar[A_HY:A_HY + D, lanes] + r
        if final:
            o_ref[:, lanes] = r.astype(o_ref.dtype)
        else:
            ar[A_HY:A_HY + D, lanes] = r

    y_round(0, 512, 0, 1, False)
    y_round(512, 1024, 0, 1, False)
    y_round(1536, 1792, 0, 2, False)
    y_round(1024, 1536, 0, 1, True)
    y_round(0, 512, 1, 2, False)
    y_round(512, 1024, 1, 2, False)
    y_round(1024, 1536, 1, 2, True)
    assert vs['next'] == NMS, (vs['next'], NMS)

    @pl.when(unsafe)
    def _():
        def head(h, carry):
            t, j = h // 4, h % 4
            qt = qT_s[t, :, pl.ds(pl.multiple_of(i * TQ, TQ), TQ)]
            row = lax.broadcasted_iota(jnp.int32, qt.shape, 0)
            qt = jnp.where((row >= j * NP) & (row < (j + 1) * NP), qt, jnp.zeros_like(qt))
            qm = jnp.concatenate([upk(qt), jnp.zeros((16, TQ), bf16)], axis=0)

            def scores(c, mx):
                s = dot(upk(k_s[t, pl.ds(pl.multiple_of(c * (KC // 2), KC // 2), KC // 2), :]), qm)
                fs_s[pl.ds(pl.multiple_of(c * KC, KC), KC), :] = s
                return jnp.maximum(mx, fold8(s, jnp.max))
            mx = lax.fori_loop(0, NC, scores, jnp.full((8, TQ), -jnp.inf, f32))
            m = jnp.max(mx, axis=0, keepdims=True)

            def mix(c, acc):
                keys = pl.ds(pl.multiple_of(c * KC, KC), KC)
                p = jnp.exp2(fs_s[keys, :] - m).astype(bf16)
                return acc + dot(upk(vT_s[h, :, keys]), p)
            acc = lax.fori_loop(0, NC, mix, jnp.zeros((HP, TQ), f32))
            oT_s[h] = pk((acc * (1.0 / acc[DH:DH + 1, :])).astype(bf16))
            return carry
        lax.fori_loop(0, H, head, 0)

        def tile(n, carry):
            lanes = pl.ds(pl.multiple_of(n * 128, 128), 128)
            xcols = pl.ds(pl.multiple_of(i * TQ + n * 128, 128), 128)
            oT = upk(oT_s[:, :, lanes].reshape(H * HP // 2, 128))
            hT = xT_ref[:, xcols].astype(f32) + dot(upk(woT_s[...]), oT)
            hc = hT - jnp.mean(hT, axis=0, keepdims=True)
            hn = hc * lax.rsqrt(jnp.mean(hc * hc, axis=0, keepdims=True) + EPS)
            hn = jnp.concatenate([hn, first_row(16, 128)], axis=0).astype(bf16)
            a = jnp.maximum(dot(upk(w1T_s[:, 0:D + 16]), hn), 0.0)
            y = dot(w2T_ref[...], (a * a).astype(bf16))
            o_ref[:, lanes] = (hT + y + b2c_s[...]).astype(o_ref.dtype)
            return carry
        lax.fori_loop(0, NT, tile, 0)


@jax.jit
def pallas_sequential_preLN__mha_block__dense_activation_squared_relu__prompt_kernel(A_x, A_wqkv, A_wo, B_x, B_w1, B_b1, B_w2, B_b2):
    hbm = pl.BlockSpec(memory_space=pl.ANY)
    outT = pl.pallas_call(
        kernel,
        grid=(NQ,),
        in_specs=[hbm] * 7,
        out_specs=pl.BlockSpec((None, D, TQ), lambda i: (0, 0, i)),
        out_shape=jax.ShapeDtypeStruct((1, D, S), bf16),
        scratch_shapes=[
            pltpu.VMEM((D, S), bf16),
            pltpu.VMEM((D, 3 * D), bf16),
            pltpu.VMEM((D, D), bf16),
            pltpu.VMEM((D, F), bf16),
            pltpu.VMEM((F,), bf16),
            pltpu.VMEM((D, F), bf16),
            pltpu.VMEM((D,), bf16),
            pltpu.SemaphoreType.DMA((10,)),
            pltpu.VMEM((1408 // 2, DP), u32),
            pltpu.VMEM((D // 2, DP), u32),
            pltpu.VMEM((F // 2, DP), u32),
            pltpu.VMEM((D, 128), f32),
            pltpu.VMEM((4, 56, S), u32),
            pltpu.VMEM((4 * NT, S // 2, 128), u32),
            pltpu.VMEM((H, HP // 2, S), u32),
            pltpu.VMEM((A_END, TQ), f32),
            pltpu.VMEM((H, HP // 2, TQ), u32),
            pltpu.VMEM((NP, NVT, 128), u32),
            pltpu.VMEM((8, 128), u32),
            pltpu.VMEM((NVT // 128, D, 128), f32),
            pltpu.VMEM((S, TQ), f32),
            pltpu.VMEM((1, S), f32),
        ],
        compiler_params=pltpu.CompilerParams(
            dimension_semantics=("arbitrary",),
            vmem_limit_bytes=100 * 1024 * 1024),
    )(jnp.swapaxes(A_x, 1, 2), A_wqkv, A_wo, B_w1, B_b1, B_w2.T, B_b2)
    return jnp.swapaxes(outT, 1, 2)
```

```python
import math

import jax
import jax.numpy as jnp
from jax import lax
import jax.experimental.pallas as pl
import jax.experimental.pallas.tpu as pltpu

S, D, H, DH, F = 2048, 448, 16, 28, 1792
HP = 32
TQ = 256
NQ = S // TQ
NT = TQ // 128
R0 = 512
KC = 256
NC = S // KC
EPS = 1e-5
QSCALE = (DH ** -0.5) * math.log2(math.e)
f32, bf16, u32 = jnp.float32, jnp.bfloat16, jnp.uint32
DP = 512
NP = DH // 2
CROW = 4 * DH
BIG = 2.0 ** 100
TINY = 2.0 ** -40

NV = 240
RV = 2
NVP = NV // (8 * RV)
NVT = -(-NV // 128) * 128
NMS = H * NVP * NP
H0 = 5
PRE = 3
LAG = 3
TAIL = 'a00_p_p_a01_p_a10_a11_b_q_q_q'
NGR = (S - NV) // 16
GB = [n * NGR // NC for n in range(NC + 1)]
_ODD = [sum((GB[m + 1] - GB[m]) % 2 for m in range(n)) % 2 for n in range(NC)]
MCH = [(NV + 16 * GB[n], NV + 16 * GB[n + 1]) for n in range(NC)]

LAT = 130
LAT0 = 100
RATIO = 1.1
R2 = 0.8
RO = 0.7
OOFF = 100
TSTART = 100
TEND = 400
PAUSE0 = 300
PAUSE1 = 1000
P0S = 400
P0E = 250
R5R = 0.01
T_ATT = H * (8 * NGR + 32 * NC)
T_FFN = 7616

A_P = (0, S // 2)
A_PV = S
A_C = A_PV + H * NV // 2
A_HY = A_C + H * 8
A_HD = A_HY + D
A_ACT = A_HD + D
A_ACC = A_ACT + F // 2
A_QC = A_ACC + HP
A_QN = A_QC + 224
A_END = A_QN + 224


def _spread(n, segs):
    tot = sum((b - a) * r for a, b, r in segs)
    out = []
    for ms in range(n):
        w = tot * ms / n
        for a, b, r in segs:
            if w < (b - a) * r:
                out.append(a + w / r)
                break
            w -= (b - a) * r
    return out


def _ms_times():
    f2 = T_ATT + 896 + 2 * F
    to = T_ATT - PRE * NGR - 32 * LAG + OOFF
    return _spread(NMS, [(TSTART, to, 1.0), (to, T_ATT + PAUSE0, RO), (T_ATT + PAUSE1, f2 + 100, RATIO),
                         (f2 + 100, f2 + 4 * D + 100, RATIO * R2),
                         (f2 + 4 * D + 100, T_ATT + T_FFN - TEND, RATIO)])


def _p0_times(n0):
    t0 = 448 + 3 * F
    tb = t0 + 5 * F
    return _spread(n0, [(t0 + P0S, tb - P0E, 1.0), (tb + 150, t0 + 6 * F, R5R)])


def pk(x):
    return pltpu.bitcast(x, u32)


def upk(x):
    return pltpu.bitcast(x, bf16)


def asf(x):
    return lax.bitcast_convert_type(x, f32)


def asu(x):
    return lax.bitcast_convert_type(x, u32)


def dot(a, b):
    return jnp.dot(a, b, preferred_element_type=f32)


def pack_pairs(ke, ko):
    lo = asu(ke.astype(bf16).astype(f32)) >> 16
    bits = asu(ko)
    sign = bits & jnp.uint32(0x80000000)
    mag = (bits & jnp.uint32(0x7fffffff)).astype(jnp.int32)
    hi = jnp.maximum(mag - lo.astype(jnp.int32) + 0x8000, 0).astype(u32) & jnp.uint32(0x7fff0000)
    return sign | hi | lo


def _padT(w):
    r, c = w.shape
    rp, cp = -(-r // 128) * 128, -(-c // 128) * 128
    if rp != r:
        w = jnp.concatenate([w, jnp.zeros((rp - r, c), w.dtype)], axis=0)
    if cp != c:
        w = jnp.concatenate([w, jnp.zeros((rp, cp - c), w.dtype)], axis=1)
    return w.T


def first_row(rows, cols, val=1.0):
    return jnp.where(lax.broadcasted_iota(jnp.int32, (rows, cols), 0) == 0, val, 0.0)


def fold8(v, op):
    return op(v.reshape(v.shape[0] // 8, 8, v.shape[1]), axis=0)


def kernel(xT_hbm, wqkv_hbm, wo_hbm, w1_hbm, b1_hbm, w2T_hbm, b2_hbm, o_ref,
           xT_ref, wqkv_ref, wo_ref, w1_ref, b1_ref, w2T_ref, b2_ref, sems,
           wT_s, woT_s, w1T_s, b2c_s, qT_s, k_s, vT_s, ar, oT_s, kp_s, z_s, kt_s, fs_s, mu_s, qb_s):
    i = pl.program_id(0)

    def fetch_q(blk):
        cols = pl.ds(pl.multiple_of(blk * TQ, TQ), TQ)
        for t in range(4):
            ar[A_QN + 56 * t:A_QN + 56 * (t + 1), :] = asf(qT_s[t, :, cols])

    def qmask(src, h):
        t, j = divmod(h, 4)
        lo = j * DH
        w0 = (lo // 16) * 16
        w1 = -(-(lo + DH) // 16) * 16
        qt = asu(ar[src + 56 * t + w0 // 2:src + 56 * t + w1 // 2, :])
        row = lax.broadcasted_iota(jnp.int32, qt.shape, 0) + w0 // 2
        qt = jnp.where((row >= lo // 2) & (row < (lo + DH) // 2), qt, jnp.zeros_like(qt))
        parts = [jnp.zeros((w0, TQ), bf16), upk(qt), jnp.zeros((CROW - w1, TQ), bf16),
                 upk(asu(ar[A_C + 8 * h:A_C + 8 * h + 8, :]))]
        return jnp.concatenate([x for x in parts if x.shape[0]], axis=0)

    def set_shift(h, s):
        c = jnp.max(fold8(s, jnp.max), axis=0, keepdims=True).astype(bf16).astype(f32)
        c = jnp.broadcast_to(c, (8, TQ))
        row = lax.broadcasted_iota(jnp.int32, (8, TQ), 0)
        ar[A_C + 8 * h:A_C + 8 * h + 8, :] = asf(jnp.where(row == 0, asu(-c) >> 16, jnp.uint32(0)))
        return c

    def qk_chunk(qm, h, c):
        r0, r1 = MCH[c]
        rm = r0 + 16 * (((r1 - r0) // 16 + (_ODD[c] + h * NGR) % 2) // 2)
        halves = [jnp.concatenate([dot(upk(k_s[4 * n + h // 4, a // 2:b // 2, :]), qm[:, n * 128:(n + 1) * 128])
                                   for n in range(NT)], axis=1) for a, b in ((r0, rm), (rm, r1))]
        p = jnp.exp2(jnp.concatenate(halves, axis=0)).astype(bf16)
        ar[A_P[h % 2] + r0 // 2:A_P[h % 2] + r1 // 2, :] = asf(pk(p))
        return halves[0]

    def make_stream(seq, after, prebuilt, times, free, lat):
        vs = dict(next=0, free=free, shift=set(), done=set())
        on = z_s[...] == 0
        on_k = jnp.broadcast_to(on[None], (RV, 8, 128))
        on_q = jnp.concatenate([on] * NT, axis=1)
        toks = []
        clk = dict(now=0)

        def gate(v, tok):
            if tok is None:
                return v
            if v.ndim not in tok[4]:
                t = tok[1][tok[2]:tok[2] + 8, tok[3]:tok[3] + 128]
                tok[4][v.ndim] = (jnp.broadcast_to(t, v.shape) if v.ndim == 3
                                  else jnp.concatenate([t] * NT, axis=1))
            return lax.select(on_k if v.ndim == 3 else on_q, v, tok[4][v.ndim])

        def qb_build(h, src, p, tok):
            rw = 56 * (h // 4) + (h % 4) * NP + p
            qt = gate(ar[src + rw // 8 * 8:src + rw // 8 * 8 + 8, :], tok)
            qq = asu(jnp.broadcast_to(qt[rw % 8:rw % 8 + 1, :], (8, TQ)))
            qb_s[h % 2, 2 * p] = asf(qq << 16)
            qb_s[h % 2, 2 * p + 1] = asf(qq & jnp.uint32(0xffff0000))

        def tok_at(t):
            best = None
            for tok in toks:
                if tok[0] <= t and (best is None or tok[0] > best[0]):
                    best = tok
            return best

        def micro(ms):
            pos, rem = divmod(ms, NVP * NP)
            h = seq[pos][0]
            pc, p = divmod(rem, NP)
            tok = tok_at(times[ms])
            kv = gate(kp_s[p, pc * RV:(pc + 1) * RV], tok)
            w = jnp.broadcast_to(kv[:, :, h:h + 1], (RV, 8, TQ))
            for e, a in enumerate((asf(asu(w) << 16), w)):
                tt = a * qb_s[h % 2, 2 * p + e:2 * p + e + 1]
                vs['acc'] = tt if p == 0 and e == 0 else vs['acc'] + tt
            nxt = seq[pos + 1] if pos + 1 < len(seq) else after
            if rem % NVP == 0:
                qb_build(*nxt, rem // NVP, tok)
            if p == NP - 1:
                assert h in vs['free'], (h, ms)
                if pc == 0:
                    vs['c'] = set_shift(h, vs['acc'].reshape(RV * 8, TQ))
                    vs['shift'].add(h)
                pv = jnp.exp2(vs['acc'] - vs['c'][None]).reshape(RV * 8, TQ).astype(bf16)
                r0 = A_PV + (h * NV + pc * RV * 8) // 2
                ar[r0:r0 + RV * 4, :] = asf(pk(pv))
                if pc == NVP - 1:
                    vs['done'].add(h)

        def issued(res, cost, ntile=1):
            if res is not None:
                del toks[:-256]
                for n in range(ntile):
                    for u in range(res.shape[0] // 16):
                        toks.append([clk['now'] + res.shape[0] * n + 16 * u + lat, res, 16 * u, 128 * n, {}])
            clk['now'] += cost
            while vs['next'] < len(times) and times[vs['next']] < clk['now'] + lat:
                micro(vs['next'])
                vs['next'] += 1

        if not prebuilt:
            for p in range(NP):
                qb_build(*seq[0], p, None)
        return vs, issued

    @pl.when(i == 0)
    def _():
        srcs = [
            (wqkv_hbm.at[:, 0:256], wqkv_ref.at[:, 0:256]),
            (xT_hbm.at[0, :, 0:R0], xT_ref.at[:, 0:R0]),
            (wqkv_hbm.at[:, 256:512], wqkv_ref.at[:, 256:512]),
            (wqkv_hbm.at[:, 512:3 * D], wqkv_ref.at[:, 512:3 * D]),
            (xT_hbm.at[0, :, R0:S], xT_ref.at[:, R0:S]),
            (wo_hbm, wo_ref), (w1_hbm, w1_ref), (b1_hbm, b1_ref), (b2_hbm, b2_ref),
            (w2T_hbm, w2T_ref),
        ]
        cps = [pltpu.make_async_copy(a, b, sems.at[n]) for n, (a, b) in enumerate(srcs)]
        for cp in cps:
            cp.start()
        c_wa1, c_x0, c_wa2, c_wb, c_x1, c_wo, c_w1, c_b1, c_b2, c_w2 = cps
        hook, mus = [], []

        def ln_chunk(c):
            x = xT_ref[:, c * R0:(c + 1) * R0].astype(f32)
            mu = jnp.mean(x, axis=0, keepdims=True)
            mus.append(mu)
            xc = x - mu
            rs = lax.rsqrt(jnp.mean(xc * xc, axis=0, keepdims=True) + EPS)
            return xc.astype(bf16), rs

        def proj(r0, r1, xc):
            r = dot(upk(wT_s[r0 // 2:r1 // 2, 0:D]), xc)
            if hook:
                hook[0](r, (r1 - r0) * (R0 // 128), R0 // 128)
            return r

        def q_part(c, xn, ts):
            r0, r1 = 112 * ts[0], 112 * (ts[-1] + 1)
            r = proj(r0, r1, xn[0]) * (xn[1] * QSCALE)
            for t in ts:
                qT_s[t, :, c * R0:(c + 1) * R0] = pk(r[112 * t - r0:112 * (t + 1) - r0, :].astype(bf16))

        def k_part(c, xn):
            r = proj(D, 2 * D, xn[0]) * xn[1]
            if c == 0:
                for n in range(NVT // 128):
                    kt_s[n] = r[:, n * 128:(n + 1) * 128]
                for p in range(NP):
                    for n in range(NVT // 128):
                        w = pack_pairs(kt_s[n, pl.ds(2 * p, H, stride=DH), :],
                                       kt_s[n, pl.ds(2 * p + 1, H, stride=DH), :])
                        w = jnp.concatenate([w, jnp.zeros((128 - H, 128), u32)], axis=0)
                        kp_s[p, n * 16:(n + 1) * 16] = asf(w.T).reshape(16, 8, 128)
            for t in range(4):
                kt = jnp.concatenate([r[112 * t:112 * (t + 1), :], first_row(16, R0)], axis=0)
                kk = pk(kt.T.astype(bf16))
                for n in range(NT):
                    k_s[4 * n + t, c * R0 // 2:(c + 1) * R0 // 2, :] = kk

        def v_part(c, xn, hs):
            r0, r1 = DH * hs[0], DH * (hs[-1] + 1)
            r = proj(2 * D + r0, 2 * D + r1, xn[0]) * xn[1]
            for h in hs:
                blk = jnp.concatenate([r[DH * h - r0:DH * (h + 1) - r0, :], first_row(HP - DH, R0)], axis=0)
                vT_s[h, :, c * R0:(c + 1) * R0] = pk(blk.astype(bf16))

        def wt_part(c0, c1):
            wT = pk(_padT(wqkv_ref[:, c0:c1].astype(f32)).astype(bf16))
            wT_s[c0 // 2:c0 // 2 + wT.shape[0], :] = wT

        z_s[...] = jnp.zeros((8, 128), u32)
        c_wa1.wait()
        wt_part(0, 256)
        c_x0.wait()
        xn0 = ln_chunk(0)
        q_part(0, xn0, [0])
        c_wa2.wait()
        q_part(0, xn0, [1])
        wt_part(256, 512)
        q_part(0, xn0, [2])
        c_wb.wait()
        q_part(0, xn0, [3])
        wt_part(512, 3 * D)
        k_part(0, xn0)
        v_part(0, xn0, list(range(0, 12)))
        c_x1.wait()
        c_wo.wait()
        fetch_q(0)
        vs0, issued0 = make_stream([(h, A_QN) for h in range(H0)], (H0, A_QN), False,
                                   _p0_times(H0 * NVP * NP), set(range(H)), LAT0)
        hook.append(issued0)
        v_part(0, xn0, list(range(12, 16)))
        wo = wo_ref[...].astype(f32)
        parts = []
        for h in range(H):
            parts += [wo[DH * h:DH * (h + 1), :], jnp.zeros((HP - DH, D), f32)]
        woT_s[...] = pk(_padT(jnp.concatenate(parts, axis=0))[0:D, :].astype(bf16))
        xns = {}
        for c in range(1, S // R0):
            xns[c] = ln_chunk(c)
            k_part(c, xns[c])
        for c in range(1, S // R0):
            q_part(c, xns[c], [0, 1, 2, 3])
            if c == S // R0 - 1:
                c_w1.wait()
                c_b1.wait()
                c_b2.wait()
                c_w2.wait()
                mu_s[...] = jnp.concatenate(mus, axis=1)
                brow = first_row(DP - D, F, b1_ref[...].astype(f32).reshape(1, F))
                w1a = jnp.concatenate([w1_ref[...].astype(f32), brow], axis=0)
                w1T_s[...] = pk(w1a.T.astype(bf16))
            v_part(c, xns[c], list(range(H)))
        assert vs0['next'] == H0 * NVP * NP
        b2 = b2_ref[...].astype(f32).reshape(1, D)
        b2c_s[...] = _padT(jnp.broadcast_to(b2, (128, D)))[0:D, :]
        qm = qmask(A_QN, 0)
        for c in range(PRE):
            qk_chunk(qm, 0, c)

    st = dict(qm=qmask(A_QN, 0), bad=None)
    ar[A_QC:A_QC + 224, :] = ar[A_QN:A_QN + 224, :]
    fetch_q(jnp.minimum(i + 1, NQ - 1))
    vs, issued = make_stream([(h, A_QC) for h in range(H0, H)] + [(h, A_QN) for h in range(H0)],
                             (H0, A_QN), True, _ms_times(), set(range(H0, H)), LAT)

    def do_qk(n):
        hq, c = divmod(n, NC)
        if c == 0:
            assert hq < H0 or hq % H in vs['shift'], hq
            st['qm'] = qmask(A_QC if hq < H else A_QN, hq % H)
        first = qk_chunk(st['qm'], hq % H, c)
        issued(first, (MCH[c][1] - MCH[c][0]) // 2)

    def do_pv(n):
        h, pos = divmod(n, NC)
        order = [1, 2, 3, 4, 5, 6, 7, 0] if h < H - 1 else [1, 2, 3, 4, 5, 0, 6, 7]
        c = order[pos]
        base = A_P[h % 2]
        if c == 0:
            assert h < H0 or h in vs['done'], h
            p = ar[A_PV + h * NV // 2:A_PV + (h + 1) * NV // 2, :]
            if NV < KC:
                p = jnp.concatenate([p, ar[base + NV // 2:base + KC // 2, :]], axis=0)
            vs['free'].add(h)
        else:
            p = ar[base + c * KC // 2:base + (c + 1) * KC // 2, :]
        acc = dot(upk(vT_s[h, :, c * KC:(c + 1) * KC]), upk(asu(p)))
        if pos > 0:
            acc = ar[A_ACC:A_ACC + HP, :] + acc
        if pos < NC - 1:
            ar[A_ACC:A_ACC + HP, :] = acc
        else:
            l = acc[DH:DH + 1, :]
            oT_s[h] = pk((acc * (1.0 / l)).astype(bf16))
            bad = fold8(jnp.where(jnp.abs(acc) <= BIG, 0.0, 1.0), jnp.max)
            bad = jnp.maximum(bad, jnp.where(l >= TINY, 0.0, 1.0))
            st['bad'] = bad if st['bad'] is None else jnp.maximum(st['bad'], bad)
        issued(None, 32)

    shift, sums = {}, {}

    def do_op(k0, k1, n0, n1, r0, r1):
        lanes = slice(n0 * 128, n1 * 128)
        oT = upk(oT_s[k0 // HP:k1 // HP, :, lanes].reshape((k1 - k0) // 2, (n1 - n0) * 128))
        r = dot(upk(woT_s[r0 // 2:r1 // 2, k0:k1]), oT)
        issued(r, (r1 - r0) * ((k1 - k0) // 128) * (n1 - n0) // 4)
        if k0 == 0:
            xcols = pl.ds(pl.multiple_of(i * TQ + n0 * 128, 128), 128)
            shift[n0] = mu_s[0:1, xcols]
            ar[A_HD + r0:A_HD + r1, lanes] = (xT_ref[r0:r1, xcols].astype(f32) - shift[n0]) + r
        else:
            d = ar[A_HD + r0:A_HD + r1, lanes] + r
            ar[A_HD + r0:A_HD + r1, lanes] = d
            sums[r0] = (fold8(d, jnp.sum), fold8(d * d, jnp.sum))

    def ln2(n):
        lanes = slice(n * 128, (n + 1) * 128)
        s1 = sum(v[0][:, lanes] for v in sums.values())
        s2 = sum(v[1][:, lanes] for v in sums.values())
        mu = jnp.sum(s1, axis=0, keepdims=True) * (1.0 / D)
        var = jnp.maximum(jnp.sum(s2, axis=0, keepdims=True) * (1.0 / D) - mu * mu, 0.0)
        hn = (ar[A_HD:A_HD + D, lanes] - mu) * lax.rsqrt(var + EPS)
        return jnp.concatenate([hn, first_row(16, 128)], axis=0).astype(bf16)

    npv = 0
    for n in range(PRE, H * NC):
        do_qk(n)
        while npv <= n - LAG:
            do_pv(npv)
            npv += 1
    nqk = H * NC
    HD = D // 2
    for item in TAIL.split('_'):
        if item == 'q':
            do_qk(nqk)
            nqk += 1
        elif item == 'p':
            do_pv(npv)
            npv += 1
        elif item[0] == 'a':
            n, hf = int(item[1]), int(item[2])
            do_op(0, 384, n, n + 1, hf * HD, (hf + 1) * HD)
        elif item == 'b':
            assert npv == H * NC
            for hf in range(2):
                do_op(384, 512, 0, NT, hf * HD, (hf + 1) * HD)
    assert nqk == H * NC + PRE
    unsafe = jnp.max(st['bad']) > 0.0

    for n in range(NT):
        lanes = slice(n * 128, (n + 1) * 128)
        a = dot(upk(w1T_s[:, 0:D + 16]), ln2(n))
        issued(a, F)
        ar[A_HY:A_HY + D, lanes] = ar[A_HD:A_HD + D, lanes] + (b2c_s[...] + shift[n])
        a = jnp.maximum(a, 0.0)
        ar[A_ACT:A_ACT + F // 2, lanes] = asf(pk((a * a).astype(bf16)))

    def y_round(k0, k1, n0, n1, final):
        lanes = slice(n0 * 128, n1 * 128)
        r = dot(w2T_ref[:, k0:k1], upk(asu(ar[A_ACT + k0 // 2:A_ACT + k1 // 2, lanes])))
        issued(r, D)
        r = ar[A_HY:A_HY + D, lanes] + r
        if final:
            o_ref[:, lanes] = r.astype(o_ref.dtype)
        else:
            ar[A_HY:A_HY + D, lanes] = r

    y_round(0, 512, 0, 1, False)
    y_round(512, 1024, 0, 1, False)
    y_round(1536, 1792, 0, 2, False)
    y_round(1024, 1536, 0, 1, True)
    y_round(0, 512, 1, 2, False)
    y_round(512, 1024, 1, 2, False)
    y_round(1024, 1536, 1, 2, True)
    assert vs['next'] == NMS, (vs['next'], NMS)

    @pl.when(unsafe)
    def _():
        def head(h, carry):
            t, j = h // 4, h % 4
            qt = qT_s[t, :, pl.ds(pl.multiple_of(i * TQ, TQ), TQ)]
            row = lax.broadcasted_iota(jnp.int32, qt.shape, 0)
            qt = jnp.where((row >= j * NP) & (row < (j + 1) * NP), qt, jnp.zeros_like(qt))
            qm = jnp.concatenate([upk(qt), jnp.zeros((16, TQ), bf16)], axis=0)

            def scores(c, mx):
                s = dot(upk(k_s[t, pl.ds(pl.multiple_of(c * (KC // 2), KC // 2), KC // 2), :]), qm)
                fs_s[pl.ds(pl.multiple_of(c * KC, KC), KC), :] = s
                return jnp.maximum(mx, fold8(s, jnp.max))
            mx = lax.fori_loop(0, NC, scores, jnp.full((8, TQ), -jnp.inf, f32))
            m = jnp.max(mx, axis=0, keepdims=True)

            def mix(c, acc):
                keys = pl.ds(pl.multiple_of(c * KC, KC), KC)
                p = jnp.exp2(fs_s[keys, :] - m).astype(bf16)
                return acc + dot(upk(vT_s[h, :, keys]), p)
            acc = lax.fori_loop(0, NC, mix, jnp.zeros((HP, TQ), f32))
            oT_s[h] = pk((acc * (1.0 / acc[DH:DH + 1, :])).astype(bf16))
            return carry
        lax.fori_loop(0, H, head, 0)

        def tile(n, carry):
            lanes = pl.ds(pl.multiple_of(n * 128, 128), 128)
            xcols = pl.ds(pl.multiple_of(i * TQ + n * 128, 128), 128)
            oT = upk(oT_s[:, :, lanes].reshape(H * HP // 2, 128))
            hT = xT_ref[:, xcols].astype(f32) + dot(upk(woT_s[...]), oT)
            hc = hT - jnp.mean(hT, axis=0, keepdims=True)
            hn = hc * lax.rsqrt(jnp.mean(hc * hc, axis=0, keepdims=True) + EPS)
            hn = jnp.concatenate([hn, first_row(16, 128)], axis=0).astype(bf16)
            a = jnp.maximum(dot(upk(w1T_s[:, 0:D + 16]), hn), 0.0)
            y = dot(w2T_ref[...], (a * a).astype(bf16))
            o_ref[:, lanes] = (hT + y + b2c_s[...]).astype(o_ref.dtype)
            return carry
        lax.fori_loop(0, NT, tile, 0)


@jax.jit
def pallas_sequential_preLN__mha_block__dense_activation_squared_relu__prompt_kernel(A_x, A_wqkv, A_wo, B_x, B_w1, B_b1, B_w2, B_b2):
    hbm = pl.BlockSpec(memory_space=pl.ANY)
    outT = pl.pallas_call(
        kernel,
        grid=(NQ,),
        in_specs=[hbm] * 7,
        out_specs=pl.BlockSpec((None, D, TQ), lambda i: (0, 0, i)),
        out_shape=jax.ShapeDtypeStruct((1, D, S), bf16),
        scratch_shapes=[
            pltpu.VMEM((D, S), bf16),
            pltpu.VMEM((D, 3 * D), bf16),
            pltpu.VMEM((D, D), bf16),
            pltpu.VMEM((D, F), bf16),
            pltpu.VMEM((F,), bf16),
            pltpu.VMEM((D, F), bf16),
            pltpu.VMEM((D,), bf16),
            pltpu.SemaphoreType.DMA((10,)),
            pltpu.VMEM((1408 // 2, DP), u32),
            pltpu.VMEM((D // 2, DP), u32),
            pltpu.VMEM((F // 2, DP), u32),
            pltpu.VMEM((D, 128), f32),
            pltpu.VMEM((4, 56, S), u32),
            pltpu.VMEM((4 * NT, S // 2, 128), u32),
            pltpu.VMEM((H, HP // 2, S), u32),
            pltpu.VMEM((A_END, TQ), f32),
            pltpu.VMEM((H, HP // 2, TQ), u32),
            pltpu.VMEM((NP, NVT // 8, 8, 128), f32),
            pltpu.VMEM((8, 128), u32),
            pltpu.VMEM((NVT // 128, D, 128), f32),
            pltpu.VMEM((S, TQ), f32),
            pltpu.VMEM((1, S), f32),
            pltpu.VMEM((2, DH, 8, TQ), f32),
        ],
        compiler_params=pltpu.CompilerParams(
            dimension_semantics=("arbitrary",),
            vmem_limit_bytes=100 * 1024 * 1024),
    )(jnp.swapaxes(A_x, 1, 2), A_wqkv, A_wo, B_w1, B_b1, B_w2.T, B_b2)
    return jnp.swapaxes(outT, 1, 2)
```

```python
import math

import jax
import jax.numpy as jnp
from jax import lax
import jax.experimental.pallas as pl
import jax.experimental.pallas.tpu as pltpu

S, D, H, DH, F = 2048, 448, 16, 28, 1792
HP = 32
TQ = 256
NQ = S // TQ
NT = TQ // 128
R0 = 512
KC = 256
NC = S // KC
EPS = 1e-5
QSCALE = (DH ** -0.5) * math.log2(math.e)
f32, bf16, u32 = jnp.float32, jnp.bfloat16, jnp.uint32
DP = 512
NP = DH // 2
CROW = 4 * DH
BIG = 2.0 ** 100
TINY = 2.0 ** -40

NV = 240
RV = 2
NVP = NV // (8 * RV)
NVT = -(-NV // 128) * 128
NMS = H * NVP * NP
H0 = 5
PRE = 3
LAG = 3
TAIL = 'a00_p_p_a01_p_a10_a11_b_q_q_q'
NGR = (S - NV) // 16
GB = [n * NGR // NC for n in range(NC + 1)]
_ODD = [sum((GB[m + 1] - GB[m]) % 2 for m in range(n)) % 2 for n in range(NC)]
MCH = [(NV + 16 * GB[n], NV + 16 * GB[n + 1]) for n in range(NC)]

LAT = 130
LAT0 = 100
RATIO = 1.1
R2 = 0.8
RO = 0.7
OOFF = 100
TSTART = 100
TEND = 400
PAUSE0 = 300
PAUSE1 = 1000
P0S = 400
P0E = 250
R5R = 0.01
T_ATT = H * (8 * NGR + 32 * NC)
T_FFN = 7616

A_P = (0, S // 2)
A_PV = S
A_C = A_PV + H * NV // 2
A_HY = A_C + H * 8
A_HD = A_HY + D
A_ACT = A_HD + D
A_ACC = A_ACT + F // 2
A_QC = A_ACC + HP
A_QN = A_QC + 224
A_END = A_QN + 224


def _spread(n, segs):
    tot = sum((b - a) * r for a, b, r in segs)
    out = []
    for ms in range(n):
        w = tot * ms / n
        for a, b, r in segs:
            if w < (b - a) * r:
                out.append(a + w / r)
                break
            w -= (b - a) * r
    return out


def _ms_times():
    f2 = T_ATT + 896 + 2 * F
    to = T_ATT - PRE * NGR - 32 * LAG + OOFF
    return _spread(NMS, [(TSTART, to, 1.0), (to, T_ATT + PAUSE0, RO), (T_ATT + PAUSE1, f2 + 100, RATIO),
                         (f2 + 100, f2 + 4 * D + 100, RATIO * R2),
                         (f2 + 4 * D + 100, T_ATT + T_FFN - TEND, RATIO)])


def _p0_times(n0):
    t0 = 448 + 3 * F
    tb = t0 + 5 * F
    return _spread(n0, [(t0 + P0S, tb - P0E, 1.0), (tb + 150, t0 + 6 * F, R5R)])


def pk(x):
    return pltpu.bitcast(x, u32)


def upk(x):
    return pltpu.bitcast(x, bf16)


def asf(x):
    return lax.bitcast_convert_type(x, f32)


def asu(x):
    return lax.bitcast_convert_type(x, u32)


def dot(a, b):
    return jnp.dot(a, b, preferred_element_type=f32)


def pack_pairs(ke, ko):
    lo = asu(ke.astype(bf16).astype(f32)) >> 16
    bits = asu(ko)
    sign = bits & jnp.uint32(0x80000000)
    mag = (bits & jnp.uint32(0x7fffffff)).astype(jnp.int32)
    hi = jnp.maximum(mag - lo.astype(jnp.int32) + 0x8000, 0).astype(u32) & jnp.uint32(0x7fff0000)
    return sign | hi | lo


def _padT(w):
    r, c = w.shape
    rp, cp = -(-r // 128) * 128, -(-c // 128) * 128
    if rp != r:
        w = jnp.concatenate([w, jnp.zeros((rp - r, c), w.dtype)], axis=0)
    if cp != c:
        w = jnp.concatenate([w, jnp.zeros((rp, cp - c), w.dtype)], axis=1)
    return w.T


def first_row(rows, cols, val=1.0):
    return jnp.where(lax.broadcasted_iota(jnp.int32, (rows, cols), 0) == 0, val, 0.0)


def fold8(v, op):
    return op(v.reshape(v.shape[0] // 8, 8, v.shape[1]), axis=0)


def kernel(xT_hbm, wqkv_hbm, wo_hbm, w1_hbm, b1_hbm, w2T_hbm, b2_hbm, o_ref,
           xT_ref, wqkv_ref, wo_ref, w1_ref, b1_ref, w2T_ref, b2_ref, sems,
           wT_s, woT_s, w1T_s, b2c_s, qT_s, k_s, vT_s, ar, oT_s, kp_s, z_s, kt_s, fs_s, mu_s, qb_s):
    i = pl.program_id(0)

    def fetch_q(blk):
        cols = pl.ds(pl.multiple_of(blk * TQ, TQ), TQ)
        for t in range(4):
            ar[A_QN + 56 * t:A_QN + 56 * (t + 1), :] = asf(qT_s[t, :, cols])

    def qmask(src, h):
        t, j = divmod(h, 4)
        lo = j * DH
        w0 = (lo // 16) * 16
        w1 = -(-(lo + DH) // 16) * 16
        qt = asu(ar[src + 56 * t + w0 // 2:src + 56 * t + w1 // 2, :])
        row = lax.broadcasted_iota(jnp.int32, qt.shape, 0) + w0 // 2
        qt = jnp.where((row >= lo // 2) & (row < (lo + DH) // 2), qt, jnp.zeros_like(qt))
        parts = [jnp.zeros((w0, TQ), bf16)] if w0 else []
        parts.append(upk(qt))
        if w1 < CROW:
            parts.append(jnp.zeros((CROW - w1, TQ), bf16))
        parts.append(upk(asu(ar[A_C + 8 * h:A_C + 8 * h + 8, :])))
        return jnp.concatenate(parts, axis=0)

    def set_shift(h, s):
        c = jnp.max(fold8(s, jnp.max), axis=0, keepdims=True).astype(bf16).astype(f32)
        c = jnp.broadcast_to(c, (8, TQ))
        row = lax.broadcasted_iota(jnp.int32, (8, TQ), 0)
        ar[A_C + 8 * h:A_C + 8 * h + 8, :] = asf(jnp.where(row == 0, asu(-c) >> 16, jnp.uint32(0)))
        return c

    def qk_chunk(qm, h, c):
        r0, r1 = MCH[c]
        rm = r0 + 16 * (((r1 - r0) // 16 + (_ODD[c] + h * NGR) % 2) // 2)
        halves = [jnp.concatenate([dot(upk(k_s[4 * n + h // 4, a // 2:b // 2, :]), qm[:, n * 128:(n + 1) * 128])
                                   for n in range(NT)], axis=1) for a, b in ((r0, rm), (rm, r1))]
        p = jnp.exp2(jnp.concatenate(halves, axis=0)).astype(bf16)
        ar[A_P[h % 2] + r0 // 2:A_P[h % 2] + r1 // 2, :] = asf(pk(p))
        return halves[0]

    def make_stream(seq, after, prebuilt, times, free, lat):
        vs = dict(next=0, free=free, shift=set(), done=set())
        on = z_s[...] == 0
        on_k = jnp.broadcast_to(on[None], (RV, 8, 128))
        on_q = jnp.concatenate([on] * NT, axis=1)
        toks = []
        clk = dict(now=0)

        def gate(v, tok):
            if tok is None:
                return v
            if v.ndim not in tok[4]:
                t = tok[1][tok[2]:tok[2] + 8, tok[3]:tok[3] + 128]
                tok[4][v.ndim] = (jnp.broadcast_to(t, v.shape) if v.ndim == 3
                                  else jnp.concatenate([t] * NT, axis=1))
            return lax.select(on_k if v.ndim == 3 else on_q, v, tok[4][v.ndim])

        def qb_build(h, src, p, tok):
            rw = 56 * (h // 4) + (h % 4) * NP + p
            qt = gate(ar[src + rw // 8 * 8:src + rw // 8 * 8 + 8, :], tok)
            qq = asu(jnp.broadcast_to(qt[rw % 8:rw % 8 + 1, :], (8, TQ)))
            qb_s[h % 2, 2 * p] = asf(qq << 16)
            qb_s[h % 2, 2 * p + 1] = asf(qq & jnp.uint32(0xffff0000))

        def tok_at(t):
            best = None
            for tok in toks:
                if tok[0] <= t and (best is None or tok[0] > best[0]):
                    best = tok
            return best

        def micro(ms):
            pos, rem = divmod(ms, NVP * NP)
            h = seq[pos][0]
            pc, p = divmod(rem, NP)
            tok = tok_at(times[ms])
            kv = gate(kp_s[p, pc * RV:(pc + 1) * RV], tok)
            w = jnp.broadcast_to(kv[:, :, h:h + 1], (RV, 8, TQ))
            for e, a in enumerate((asf(asu(w) << 16), w)):
                tt = a * qb_s[h % 2, 2 * p + e:2 * p + e + 1]
                vs['acc'] = tt if p == 0 and e == 0 else vs['acc'] + tt
            nxt = seq[pos + 1] if pos + 1 < len(seq) else after
            if rem % NVP == 0:
                qb_build(*nxt, rem // NVP, tok)
            if p == NP - 1:
                assert h in vs['free'], (h, ms)
                if pc == 0:
                    vs['c'] = set_shift(h, vs['acc'].reshape(RV * 8, TQ))
                    vs['shift'].add(h)
                pv = jnp.exp2(vs['acc'] - vs['c'][None]).reshape(RV * 8, TQ).astype(bf16)
                r0 = A_PV + (h * NV + pc * RV * 8) // 2
                ar[r0:r0 + RV * 4, :] = asf(pk(pv))
                if pc == NVP - 1:
                    vs['done'].add(h)

        def issued(res, cost, ntile=1):
            if res is not None:
                del toks[:-256]
                for n in range(ntile):
                    for u in range(res.shape[0] // 16):
                        toks.append([clk['now'] + res.shape[0] * n + 16 * u + lat, res, 16 * u, 128 * n, {}])
            clk['now'] += cost
            while vs['next'] < len(times) and times[vs['next']] < clk['now'] + lat:
                micro(vs['next'])
                vs['next'] += 1

        if not prebuilt:
            for p in range(NP):
                qb_build(*seq[0], p, None)
        return vs, issued

    @pl.when(i == 0)
    def _():
        srcs = [
            (wqkv_hbm.at[:, 0:256], wqkv_ref.at[:, 0:256]),
            (xT_hbm.at[0, :, 0:R0], xT_ref.at[:, 0:R0]),
            (wqkv_hbm.at[:, 256:512], wqkv_ref.at[:, 256:512]),
            (wqkv_hbm.at[:, 512:3 * D], wqkv_ref.at[:, 512:3 * D]),
            (xT_hbm.at[0, :, R0:S], xT_ref.at[:, R0:S]),
            (wo_hbm, wo_ref), (w1_hbm, w1_ref), (b1_hbm, b1_ref), (b2_hbm, b2_ref),
            (w2T_hbm, w2T_ref),
        ]
        cps = [pltpu.make_async_copy(a, b, sems.at[n]) for n, (a, b) in enumerate(srcs)]
        for cp in cps:
            cp.start()
        c_wa1, c_x0, c_wa2, c_wb, c_x1, c_wo, c_w1, c_b1, c_b2, c_w2 = cps
        hook, mus = [], []

        def ln_chunk(c):
            x = xT_ref[:, c * R0:(c + 1) * R0].astype(f32)
            mu = jnp.mean(x, axis=0, keepdims=True)
            mus.append(mu)
            xc = x - mu
            rs = lax.rsqrt(jnp.mean(xc * xc, axis=0, keepdims=True) + EPS)
            return xc.astype(bf16), rs

        def proj(r0, r1, xc):
            r = dot(upk(wT_s[r0 // 2:r1 // 2, 0:D]), xc)
            if hook:
                hook[0](r, (r1 - r0) * (R0 // 128), R0 // 128)
            return r

        def q_part(c, xn, ts):
            r0, r1 = 112 * ts[0], 112 * (ts[-1] + 1)
            r = proj(r0, r1, xn[0]) * (xn[1] * QSCALE)
            for t in ts:
                qT_s[t, :, c * R0:(c + 1) * R0] = pk(r[112 * t - r0:112 * (t + 1) - r0, :].astype(bf16))

        def k_part(c, xn):
            r = proj(D, 2 * D, xn[0]) * xn[1]
            if c == 0:
                for n in range(NVT // 128):
                    kt_s[n] = r[:, n * 128:(n + 1) * 128]
                for p in range(NP):
                    for n in range(NVT // 128):
                        w = pack_pairs(kt_s[n, pl.ds(2 * p, H, stride=DH), :],
                                       kt_s[n, pl.ds(2 * p + 1, H, stride=DH), :])
                        w = jnp.concatenate([w, jnp.zeros((128 - H, 128), u32)], axis=0)
                        kp_s[p, n * 16:(n + 1) * 16] = asf(w.T).reshape(16, 8, 128)
            for t in range(4):
                kt = jnp.concatenate([r[112 * t:112 * (t + 1), :], first_row(16, R0)], axis=0)
                kk = pk(kt.T.astype(bf16))
                for n in range(NT):
                    k_s[4 * n + t, c * R0 // 2:(c + 1) * R0 // 2, :] = kk

        def v_part(c, xn, hs):
            r0, r1 = DH * hs[0], DH * (hs[-1] + 1)
            r = proj(2 * D + r0, 2 * D + r1, xn[0]) * xn[1]
            for h in hs:
                blk = jnp.concatenate([r[DH * h - r0:DH * (h + 1) - r0, :], first_row(HP - DH, R0)], axis=0)
                vT_s[h, :, c * R0:(c + 1) * R0] = pk(blk.astype(bf16))

        def wt_part(c0, c1):
            wT = pk(_padT(wqkv_ref[:, c0:c1].astype(f32)).astype(bf16))
            wT_s[c0 // 2:c0 // 2 + wT.shape[0], :] = wT

        z_s[...] = jnp.zeros((8, 128), u32)
        c_wa1.wait()
        wt_part(0, 256)
        c_x0.wait()
        xn0 = ln_chunk(0)
        q_part(0, xn0, [0])
        c_wa2.wait()
        q_part(0, xn0, [1])
        wt_part(256, 512)
        q_part(0, xn0, [2])
        c_wb.wait()
        q_part(0, xn0, [3])
        wt_part(512, 3 * D)
        k_part(0, xn0)
        v_part(0, xn0, list(range(0, 12)))
        c_x1.wait()
        c_wo.wait()
        fetch_q(0)
        vs0, issued0 = make_stream([(h, A_QN) for h in range(H0)], (H0, A_QN), False,
                                   _p0_times(H0 * NVP * NP), set(range(H)), LAT0)
        hook.append(issued0)
        v_part(0, xn0, list(range(12, 16)))
        wo = wo_ref[...].astype(f32)
        parts = []
        for h in range(H):
            parts += [wo[DH * h:DH * (h + 1), :], jnp.zeros((HP - DH, D), f32)]
        woT_s[...] = pk(_padT(jnp.concatenate(parts, axis=0))[0:D, :].astype(bf16))
        xns = {}
        for c in range(1, S // R0):
            xns[c] = ln_chunk(c)
            k_part(c, xns[c])
        for c in range(1, S // R0):
            q_part(c, xns[c], [0, 1, 2, 3])
            if c == S // R0 - 1:
                c_w1.wait()
                c_b1.wait()
                c_b2.wait()
                c_w2.wait()
                mu_s[...] = jnp.concatenate(mus, axis=1)
                brow = first_row(DP - D, F, b1_ref[...].astype(f32).reshape(1, F))
                w1a = jnp.concatenate([w1_ref[...].astype(f32), brow], axis=0)
                w1T_s[...] = pk(w1a.T.astype(bf16))
            v_part(c, xns[c], list(range(H)))
        assert vs0['next'] == H0 * NVP * NP
        b2 = b2_ref[...].astype(f32).reshape(1, D)
        b2c_s[...] = _padT(jnp.broadcast_to(b2, (128, D)))[0:D, :]
        qm = qmask(A_QN, 0)
        for c in range(PRE):
            qk_chunk(qm, 0, c)

    st = dict(qm=qmask(A_QN, 0), bad=None)
    ar[A_QC:A_QC + 224, :] = ar[A_QN:A_QN + 224, :]
    fetch_q(jnp.minimum(i + 1, NQ - 1))
    vs, issued = make_stream([(h, A_QC) for h in range(H0, H)] + [(h, A_QN) for h in range(H0)],
                             (H0, A_QN), True, _ms_times(), set(range(H0, H)), LAT)

    def do_qk(n):
        hq, c = divmod(n, NC)
        if c == 0:
            assert hq < H0 or hq % H in vs['shift'], hq
            st['qm'] = qmask(A_QC if hq < H else A_QN, hq % H)
        first = qk_chunk(st['qm'], hq % H, c)
        issued(first, (MCH[c][1] - MCH[c][0]) // 2)

    def do_pv(n):
        h, pos = divmod(n, NC)
        order = [1, 2, 3, 4, 5, 6, 7, 0] if h < H - 1 else [1, 2, 3, 4, 5, 0, 6, 7]
        c = order[pos]
        base = A_P[h % 2]
        if c == 0:
            assert h < H0 or h in vs['done'], h
            p = ar[A_PV + h * NV // 2:A_PV + (h + 1) * NV // 2, :]
            if NV < KC:
                p = jnp.concatenate([p, ar[base + NV // 2:base + KC // 2, :]], axis=0)
            vs['free'].add(h)
        else:
            p = ar[base + c * KC // 2:base + (c + 1) * KC // 2, :]
        acc = dot(upk(vT_s[h, :, c * KC:(c + 1) * KC]), upk(asu(p)))
        if pos > 0:
            acc = ar[A_ACC:A_ACC + HP, :] + acc
        if pos < NC - 1:
            ar[A_ACC:A_ACC + HP, :] = acc
        else:
            l = acc[DH:DH + 1, :]
            oT_s[h] = pk((acc * (1.0 / l)).astype(bf16))
            bad = fold8(jnp.where(jnp.abs(acc) <= BIG, 0.0, 1.0), jnp.max)
            bad = jnp.maximum(bad, jnp.where(l >= TINY, 0.0, 1.0))
            st['bad'] = bad if st['bad'] is None else jnp.maximum(st['bad'], bad)
        issued(None, 32)

    shift, sums = {}, {}

    def do_op(k0, k1, n0, n1, r0, r1):
        lanes = slice(n0 * 128, n1 * 128)
        oT = upk(oT_s[k0 // HP:k1 // HP, :, lanes].reshape((k1 - k0) // 2, (n1 - n0) * 128))
        r = dot(upk(woT_s[r0 // 2:r1 // 2, k0:k1]), oT)
        issued(r, (r1 - r0) * ((k1 - k0) // 128) * (n1 - n0) // 4)
        if k0 == 0:
            xcols = pl.ds(pl.multiple_of(i * TQ + n0 * 128, 128), 128)
            shift[n0] = mu_s[0:1, xcols]
            ar[A_HD + r0:A_HD + r1, lanes] = (xT_ref[r0:r1, xcols].astype(f32) - shift[n0]) + r
        else:
            d = ar[A_HD + r0:A_HD + r1, lanes] + r
            ar[A_HD + r0:A_HD + r1, lanes] = d
            sums[r0] = (fold8(d, jnp.sum), fold8(d * d, jnp.sum))

    def ln2(n):
        lanes = slice(n * 128, (n + 1) * 128)
        s1 = sum(v[0][:, lanes] for v in sums.values())
        s2 = sum(v[1][:, lanes] for v in sums.values())
        mu = jnp.sum(s1, axis=0, keepdims=True) * (1.0 / D)
        var = jnp.maximum(jnp.sum(s2, axis=0, keepdims=True) * (1.0 / D) - mu * mu, 0.0)
        hn = (ar[A_HD:A_HD + D, lanes] - mu) * lax.rsqrt(var + EPS)
        return jnp.concatenate([hn, first_row(16, 128)], axis=0).astype(bf16)

    npv = 0
    for n in range(PRE, H * NC):
        do_qk(n)
        while npv <= n - LAG:
            do_pv(npv)
            npv += 1
    nqk = H * NC
    HD = D // 2
    for item in TAIL.split('_'):
        if item == 'q':
            do_qk(nqk)
            nqk += 1
        elif item == 'p':
            do_pv(npv)
            npv += 1
        elif item[0] == 'a':
            n, hf = int(item[1]), int(item[2])
            do_op(0, 384, n, n + 1, hf * HD, (hf + 1) * HD)
        elif item == 'b':
            assert npv == H * NC
            for hf in range(2):
                do_op(384, 512, 0, NT, hf * HD, (hf + 1) * HD)
    assert nqk == H * NC + PRE
    unsafe = jnp.max(st['bad']) > 0.0

    for n in range(NT):
        lanes = slice(n * 128, (n + 1) * 128)
        a = dot(upk(w1T_s[:, 0:D + 16]), ln2(n))
        issued(a, F)
        ar[A_HY:A_HY + D, lanes] = ar[A_HD:A_HD + D, lanes] + (b2c_s[...] + shift[n])
        a = jnp.maximum(a, 0.0)
        ar[A_ACT:A_ACT + F // 2, lanes] = asf(pk((a * a).astype(bf16)))

    def y_round(k0, k1, n0, n1, final):
        lanes = slice(n0 * 128, n1 * 128)
        r = dot(w2T_ref[:, k0:k1], upk(asu(ar[A_ACT + k0 // 2:A_ACT + k1 // 2, lanes])))
        issued(r, D)
        r = ar[A_HY:A_HY + D, lanes] + r
        if final:
            o_ref[:, lanes] = r.astype(o_ref.dtype)
        else:
            ar[A_HY:A_HY + D, lanes] = r

    y_round(0, 512, 0, 1, False)
    y_round(512, 1024, 0, 1, False)
    y_round(1536, 1792, 0, 2, False)
    y_round(1024, 1536, 0, 1, True)
    y_round(0, 512, 1, 2, False)
    y_round(512, 1024, 1, 2, False)
    y_round(1024, 1536, 1, 2, True)
    assert vs['next'] == NMS, (vs['next'], NMS)

    @pl.when(unsafe)
    def _():
        def head(h, carry):
            t, j = h // 4, h % 4
            qt = qT_s[t, :, pl.ds(pl.multiple_of(i * TQ, TQ), TQ)]
            row = lax.broadcasted_iota(jnp.int32, qt.shape, 0)
            qt = jnp.where((row >= j * NP) & (row < (j + 1) * NP), qt, jnp.zeros_like(qt))
            qm = jnp.concatenate([upk(qt), jnp.zeros((16, TQ), bf16)], axis=0)

            def scores(c, mx):
                s = dot(upk(k_s[t, pl.ds(pl.multiple_of(c * (KC // 2), KC // 2), KC // 2), :]), qm)
                fs_s[pl.ds(pl.multiple_of(c * KC, KC), KC), :] = s
                return jnp.maximum(mx, fold8(s, jnp.max))
            mx = lax.fori_loop(0, NC, scores, jnp.full((8, TQ), -jnp.inf, f32))
            m = jnp.max(mx, axis=0, keepdims=True)

            def mix(c, acc):
                keys = pl.ds(pl.multiple_of(c * KC, KC), KC)
                p = jnp.exp2(fs_s[keys, :] - m).astype(bf16)
                return acc + dot(upk(vT_s[h, :, keys]), p)
            acc = lax.fori_loop(0, NC, mix, jnp.zeros((HP, TQ), f32))
            oT_s[h] = pk((acc * (1.0 / acc[DH:DH + 1, :])).astype(bf16))
            return carry
        lax.fori_loop(0, H, head, 0)

        def tile(n, carry):
            lanes = pl.ds(pl.multiple_of(n * 128, 128), 128)
            xcols = pl.ds(pl.multiple_of(i * TQ + n * 128, 128), 128)
            oT = upk(oT_s[:, :, lanes].reshape(H * HP // 2, 128))
            hT = xT_ref[:, xcols].astype(f32) + dot(upk(woT_s[...]), oT)
            hc = hT - jnp.mean(hT, axis=0, keepdims=True)
            hn = hc * lax.rsqrt(jnp.mean(hc * hc, axis=0, keepdims=True) + EPS)
            hn = jnp.concatenate([hn, first_row(16, 128)], axis=0).astype(bf16)
            a = jnp.maximum(dot(upk(w1T_s[:, 0:D + 16]), hn), 0.0)
            y = dot(w2T_ref[...], (a * a).astype(bf16))
            o_ref[:, lanes] = (hT + y + b2c_s[...]).astype(o_ref.dtype)
            return carry
        lax.fori_loop(0, NT, tile, 0)


@jax.jit
def pallas_sequential_preLN__mha_block__dense_activation_squared_relu__prompt_kernel(A_x, A_wqkv, A_wo, B_x, B_w1, B_b1, B_w2, B_b2):
    hbm = pl.BlockSpec(memory_space=pl.ANY)
    outT = pl.pallas_call(
        kernel,
        grid=(NQ,),
        in_specs=[hbm] * 7,
        out_specs=pl.BlockSpec((None, D, TQ), lambda i: (0, 0, i)),
        out_shape=jax.ShapeDtypeStruct((1, D, S), bf16),
        scratch_shapes=[
            pltpu.VMEM((D, S), bf16),
            pltpu.VMEM((D, 3 * D), bf16),
            pltpu.VMEM((D, D), bf16),
            pltpu.VMEM((D, F), bf16),
            pltpu.VMEM((F,), bf16),
            pltpu.VMEM((D, F), bf16),
            pltpu.VMEM((D,), bf16),
            pltpu.SemaphoreType.DMA((10,)),
            pltpu.VMEM((1408 // 2, DP), u32),
            pltpu.VMEM((D // 2, DP), u32),
            pltpu.VMEM((F // 2, DP), u32),
            pltpu.VMEM((D, 128), f32),
            pltpu.VMEM((4, 56, S), u32),
            pltpu.VMEM((4 * NT, S // 2, 128), u32),
            pltpu.VMEM((H, HP // 2, S), u32),
            pltpu.VMEM((A_END, TQ), f32),
            pltpu.VMEM((H, HP // 2, TQ), u32),
            pltpu.VMEM((NP, NVT // 8, 8, 128), f32),
            pltpu.VMEM((8, 128), u32),
            pltpu.VMEM((NVT // 128, D, 128), f32),
            pltpu.VMEM((S, TQ), f32),
            pltpu.VMEM((1, S), f32),
            pltpu.VMEM((2, DH, 8, TQ), f32),
        ],
        compiler_params=pltpu.CompilerParams(
            dimension_semantics=("arbitrary",),
            vmem_limit_bytes=100 * 1024 * 1024),
    )(jnp.swapaxes(A_x, 1, 2), A_wqkv, A_wo, B_w1, B_b1, B_w2.T, B_b2)
    return jnp.swapaxes(outT, 1, 2)
```
